```python
import jax
import jax.numpy as jnp

def _softmax(x, axis=-1):
    return jax.nn.softmax(x, axis=axis)
def _gelu(x):
    return jax.nn.gelu(x, approximate=True)
def _silu(x):
    return jax.nn.silu(x)
def _sigmoid(x):
    return jax.nn.sigmoid(x)
def _layernorm(x, axis=-1, eps=1e-5):
    m = jnp.mean(x, axis=axis, keepdims=True)
    v = jnp.var(x, axis=axis, keepdims=True)
    return (x - m) / jnp.sqrt(v + eps)
def _scatter_add(tgt, idx, src, axis=0):
    return tgt.at[idx].add(src)
def _segment_sum(src, seg, n):
    return jax.ops.segment_sum(src, seg, n)
class _Rng:
    def __init__(self, key):
        self._k = key
    def _next(self):
        self._k, sub = jax.random.split(self._k)
        return sub
    def normal(self, shape):
        return jax.random.normal(self._next(), shape, dtype=jnp.bfloat16)
    def randint(self, lo, hi, shape):
        return jax.random.randint(self._next(), shape, lo, hi, dtype=jnp.int32)
    def uniform(self, shape, lo=0.0, hi=1.0):
        return jax.random.uniform(self._next(), shape, jnp.bfloat16, lo, hi)
    def permutation(self, n):
        return jax.random.permutation(self._next(), n)


kernel_name = 'standalone__gqa_block_cached__near_ridge'

def _fwd_setup_inputs():
    _rng = _Rng(jax.random.key(int.from_bytes(__import__("os").urandom(4), "little")))
    _w = (lambda a: (lambda t: t.astype(jnp.bfloat16) if jnp.issubdtype(t.dtype, jnp.floating) else t)(jnp.asarray(a)))
    B, Sq, D = 16, 64, 640
    Hq, Hkv, Sk, Dh = 32, 32, 512, 192
    assert Hq % Hkv == 0, (Hq, Hkv)
    return {
        "x": _w((lambda *s: _rng.normal(s) * 0.05)(B, Sq, D)),
        "k_cache": _w((lambda *s: _rng.normal(s) * 0.05)(B, Hkv, Sk, Dh)),
        "v_cache": _w((lambda *s: _rng.normal(s) * 0.05)(B, Hkv, Sk, Dh)),
        "wq": _w((lambda *s: _rng.normal(s) * 0.05)(D, Hq * Dh) * (D ** -0.5)),
        "wo": _w((lambda *s: _rng.normal(s) * 0.05)(Hq * Dh, D) * ((Hq * Dh) ** -0.5)),
    }

def _fwd_reference(x, k_cache, v_cache, wq, wo):
    B, Sq, D = x.shape
    Hq, Dh = 32, 192
    Hkv = k_cache.shape[1]
    rep = Hq // Hkv
    q = (lambda x, *d: x.transpose(*d))((x @ wq).reshape(B, Sq, Hq, Dh), 0, 2, 1, 3)
    k = jnp.repeat(k_cache, rep, axis=1)
    v = jnp.repeat(v_cache, rep, axis=1)
    scores = jnp.einsum("bhqd,bhkd->bhqk", q, k) * (Dh ** -0.5)
    p = _softmax(scores, axis=-1)
    o = jnp.einsum("bhqk,bhkd->bhqd", p, v)
    return (lambda x, *d: x.transpose(*d))(o, 0, 2, 1, 3).reshape(B, Sq, Hq * Dh) @ wo


def setup_inputs():
    _inp = _fwd_setup_inputs()
    _gk = jax.random.fold_in(jax.random.key(int.from_bytes(__import__("os").urandom(4), "little")), 2**31 - 1)
    _shapes = [[16, 64, 640]]
    _dtypes = ['bfloat16']
    _gks = jax.random.split(_gk, len(_shapes))
    _gs = [jax.random.normal(k, s, dtype=jnp.dtype(d)) * 0.05 for k, s, d in zip(_gks, _shapes, _dtypes)]
    _inp["grad_out"] = _gs[0]
    return _inp

def reference(x, k_cache, v_cache, wq, wo, grad_out):
    _const = dict()
    def _f(*_d):
        return _fwd_reference(**{'x': _d[0], 'k_cache': _d[1], 'v_cache': _d[2], 'wq': _d[3], 'wo': _d[4], **_const})
    _out, _vjp = jax.vjp(_f, x, k_cache, v_cache, wq, wo)
    _grads = _vjp(grad_out)
    _out0 = jnp.asarray(_out)
    return (_out0, *[jnp.asarray(_g) for _g in _grads])
```

```python
import functools

import jax
import jax.numpy as jnp
import jax.experimental.pallas as pl
import jax.experimental.pallas.tpu as pltpu

_NT = (((1,), (1,)), ((), ()))
_NSLOT = 4
_W_ROWS = (48,) + (32,) * 10 + (16,)
_W_ROWS_LAST = (48,) * 8
_R_ROWS = 48
_N_INIT = 10
_NW0 = 5
_GRP = 4
_RQ = 576
_DWO_ROWS = 96
_OD_ROWS = 32
_SPLIT = 192
_PLAN = (("top", 1, 2), ("top", 1, 3), ("top", 1, 0), ("top", 1, 1), ("top", 2, 0),
         ("b2", 2, 2), ("b2", 2, 3), ("b4", 2, 1), ("b6", 3, 0), ("out", 3, 1),
         ("dwo", 3, 2), ("dwo", 3, 3))


def _dot(a, b):
    return jnp.dot(a, b, preferred_element_type=jnp.float32)


def _dot_nt(a, b):
    return jax.lax.dot_general(a, b, _NT, preferred_element_type=jnp.float32)


def _kernel(x_hbm, g_hbm, wq_hbm, wo_hbm, kt_hbm, vt_hbm,
            out_hbm, dx_hbm, dkt_hbm, dvt_hbm, dwq_hbm, dwo_hbm,
            x_sc, g_sc, xt_sc, wq_sc, wo_sc, out_acc, dx_acc, dwq_acc, dwo_acc,
            dwq_st, dwo_st, out_st, dx_st, kbuf_a, vbuf_a, kbuf_b, vbuf_b, dkbuf, dvbuf,
            sem_in, sem_out, sem_w, sem_dw, sem_misc, sem_fence,
            *, nb, sq, dh, scale, n_hp):
    n_steps = 2 * n_hp
    jl = n_steps - 1
    m = nb * sq
    hb = nb // 2
    bf16 = jnp.bfloat16
    f32 = jnp.float32
    i32 = jnp.int32
    d2 = 2 * dh
    dm = x_sc.shape[1]
    cp = pltpu.make_async_copy
    land = jnp.logical_and
    lor = jnp.logical_or

    def mult(v, k):
        return v if isinstance(v, int) else pl.multiple_of(v, k)

    def unit(j):
        return (j % 2) * nb, mult((j // 2) * d2, d2), j % _NSLOT

    bufs = ((kt_hbm, kbuf_a, 0), (vt_hbm, vbuf_a, 0), (kt_hbm, kbuf_b, hb), (vt_hbm, vbuf_b, hb))

    def kv_in(j, which=(0, 1, 2, 3), sel=slice(None)):
        b0, r0, slot = j if isinstance(j, tuple) else unit(j)
        spec = [bufs[w] + (bo, off) for w in which
                for off in range(0, d2, _R_ROWS) for bo in range(0, hb, 2)]
        return [cp(hbm.at[pl.ds(b0 + lo + bo, 2), pl.ds(mult(r0 + off, 16), _R_ROWS), :],
                   buf.at[slot, pl.ds(bo, 2), pl.ds(off, _R_ROWS), :], sem_in.at[slot])
                for hbm, buf, lo, bo, off in spec[sel]]

    def kv_in_big(j):
        b0, r0, slot = unit(j)
        return [cp(hbm.at[pl.ds(b0 + lo, hb), pl.ds(r0, d2), :], buf.at[slot], sem_in.at[slot])
                for hbm, buf, lo in bufs]

    def kv_out(j, sel=slice(None), lo=0, n=None, chunks=_W_ROWS):
        n = nb if n is None else n
        b0, r0, slot = j if isinstance(j, tuple) else unit(j)
        spec = []
        for buf, hbm in ((dkbuf, dkt_hbm), (dvbuf, dvt_hbm)):
            off = 0
            for cr in chunks:
                spec.append((buf, hbm, off, cr))
                off += cr
        return [cp(buf.at[slot, pl.ds(lo, n), pl.ds(off, cr), :],
                   hbm.at[pl.ds(b0 + lo, n), pl.ds(mult(r0 + off, 16), cr), :], sem_out.at[slot])
                for buf, hbm, off, cr in spec[sel]]

    most, rest = slice(None, -1), slice(-1, None)
    groups = ((0, hb), (hb, nb - 2 - hb), (nb - 2, 1), (nb - 1, 1))

    def last_out(gi):
        return kv_out(jl, slice(None), groups[gi][0], groups[gi][1], _W_ROWS_LAST)

    def wq_head(h, sem):
        return cp(wq_hbm.at[pl.ds(0, _RQ), pl.ds(h * d2, d2)], wq_sc.at[h, pl.ds(0, _RQ)], sem)

    def wq_bulk():
        return [wq_head(h, sem_misc.at[2]) for h in range(1, n_hp)]

    def w_in(h):
        return [cp(wo_hbm.at[h], wo_sc.at[h % 2], sem_w.at[0]),
                cp(wq_hbm.at[pl.ds(_RQ, dm - _RQ), pl.ds(mult(h * d2, d2), d2)],
                   wq_sc.at[h, pl.ds(_RQ, dm - _RQ)], sem_w.at[0])]

    def xg_in(i):
        r = pl.ds(i * m, m)
        return [cp(x_hbm.at[r], x_sc.at[r], sem_misc.at[i]),
                cp(g_hbm.at[r], g_sc.at[r], sem_misc.at[i])]

    def dw_out(h):
        return [cp(dwq_st.at[h % 2], dwq_hbm.at[:, pl.ds(mult(h * d2, d2), d2)], sem_dw.at[0])] + [
            cp(dwo_st.at[h % 2, pl.ds(r, _DWO_ROWS)], dwo_hbm.at[h, pl.ds(r, _DWO_ROWS)],
               sem_dw.at[0]) for r in range(0, d2, _DWO_ROWS)]

    def od_out(i):
        cs = []
        for o in range(i * m, (i + 1) * m, _OD_ROWS):
            r = pl.ds(o, _OD_ROWS)
            cs += [cp(out_st.at[r], out_hbm.at[r], sem_misc.at[0]),
                   cp(dx_st.at[r], dx_hbm.at[r], sem_misc.at[0])]
        return cs

    def start(cs):
        for c in cs:
            c.start()

    def start2(cs):
        for i, c in enumerate(cs):
            c.start(priority=i % 2)

    def wait(cs):
        for c in cs:
            c.wait()

    def interleave(a, b):
        r = []
        for i in range(max(len(a), len(b))):
            r += a[i:i + 1] + b[i:i + 1]
        return r

    def fence():
        pl.semaphore_signal(sem_fence.at[0], 1)
        pl.semaphore_wait(sem_fence.at[0], 1)

    def xpose(i):
        xt_sc[i] = x_sc[i * m:(i + 1) * m, :].astype(f32).T.astype(bf16)

    def cast_od(i):
        out_st[i * m:(i + 1) * m, :] = out_acc[i * m:(i + 1) * m, :].astype(bf16)
        dx_st[i * m:(i + 1) * m, :] = dx_acc[i * m:(i + 1) * m, :].astype(bf16)

    lane_lo = jax.lax.broadcasted_iota(i32, (sq, 128), 1) < 64
    lane_lo_t = jax.lax.broadcasted_iota(i32, (dh, 128), 1) < 64

    def step_sync(j):
        hp = j // 2
        r = j % 4

        @pl.when(r == 1)
        def _():
            pl.when(j >= 5)(lambda: wait(kv_out(j - 2, most)))
            start(w_in(hp + 1))
            start2(kv_in(j + 1, (0,), slice(0, _N_INIT)))

            @pl.when(j >= 5)
            def _():
                wait(dw_out(hp - 1))
                wait(kv_out(j - 4))
                wait(kv_in(j))

            @pl.when(j == 1)
            def _():
                wait(xg_in(1))
                xpose(1)
                wait(kv_in_big(1))

        @pl.when(land(r == 2, j < jl - 1))
        def _():
            wait(w_in(hp))
            start(w_in(hp + 1))
            pl.when(j == 2)(lambda: wait(wq_bulk()))
            pl.when(j >= 4)(lambda: wait(kv_out(j - 4)))
            wait(kv_in(j))

        @pl.when(land(r == 3, j < jl))
        def _():
            start(interleave(kv_out(j - 2, slice(0, _NW0)), dw_out(hp - 1)))
            pl.when(j >= 4)(lambda: wait(kv_out(j - 4, rest)))
            wait(kv_in(j))

        @pl.when(lor(land(r == 0, j >= 4), j == jl - 1))
        def _():
            pl.when(r == 0)(lambda: wait(dw_out(hp - 2)))
            start(interleave(kv_out(j - 1, slice(0, _NW0)), dw_out(hp - 1)))
            wait(kv_out(j - 4))
            wait(w_in(hp))
            wait(kv_in(j))

        @pl.when(j == jl)
        def _():
            start(kv_out(jl - 1))
            wait(kv_out(jl - 4, rest))
            cast_od(0)
            start(od_out(0))
            wait(kv_in(jl))

    def step_body(j):
        hp = j // 2
        bg = j % 2
        slot = j % _NSLOT
        rows = pl.ds(mult(bg * m, m), m)

        def kv(which, b, lo, hi):
            return bufs[which + 2 * (b // hb)][1][slot, b % hb, lo:hi, :]

        wq = wq_sc[hp]
        q = _dot(x_sc[rows, :], wq) * scale
        g = g_sc[rows, :]
        wo = wo_sc[hp % 2]
        do = _dot_nt(g, wo)

        r = j % 4
        is1 = (r == 1).astype(i32)
        is2 = land(r == 2, j < jl - 1).astype(i32)
        is3 = land(r == 3, j < jl).astype(i32)
        is0 = lor(land(r == 0, j >= 4), j == jl - 1).astype(i32)
        end_rd = (j == jl - 2).astype(i32)
        n_reg = [1]

        def issue(key, fn, n, k0=0):
            for k in range(k0, n, _GRP):
                n_reg[0] += 1
                pl.when(key * n_reg[0] == n_reg[0])(functools.partial(fn, slice(k, k + _GRP)))

        def issue_out(key, u, k0=0):
            issue(key, lambda sl: start(kv_out(u, sl)), 2 * len(_W_ROWS), k0)

        keys = {1: is1, 2: is1 + is2, 3: jnp.where(j + 3 <= jl, is1, 0)}
        units = {1: unit(j + 1), 2: unit(j + 2 + is2), 3: unit(j + 3)}
        spare = jnp.minimum(j + _NSLOT, _NSLOT)

        def point(pos, pre=None, post=None):
            todo = [(du, w) for p, du, w in _PLAN if p == pos]
            used = sorted(set(w for _, w in todo))
            for w in used if pre is not None else ():
                bufs[w][1][spare, 0, 0:16, 0:128] = pre.astype(bf16)
            for du, w in todo:
                issue(keys[du],
                      functools.partial(lambda u, w, sl: start2(kv_in(u, (w,), sl)), units[du], w),
                      (d2 // _R_ROWS) * hb // 2, _N_INIT if (du, w) == (1, 0) else 0)
            for w in used if post is not None else ():
                bufs[w][1][spare, hb - 1, d2 - 16:d2, 0:128] = post.astype(bf16)

        point("top")
        issue_out(is3 + is0, unit(j - 1 - is3), _NW0)
        issue_out(is3, unit(j - 1))

        def split(a):
            t0, t1, t2 = a[:, 0:128], a[:, 128:256], a[:, 256:384]
            a0 = jnp.concatenate([t0, jnp.where(lane_lo, t1, 0.0)], axis=1)
            a1 = jnp.concatenate([jnp.where(lane_lo, 0.0, t1), t2], axis=1)
            return a0.astype(bf16), a1.astype(bf16)

        def scores(b):
            q0, q1 = split(q[b * sq:(b + 1) * sq])
            d0, d1 = split(do[b * sq:(b + 1) * sq])
            ps = []
            dss = []
            for h, (qh, doh) in enumerate(((q0, d0), (q1, d1))):
                s = _dot(qh, kv(0, b, h * 128, h * 128 + 256))
                dp = _dot(doh, kv(1, b, h * 128, h * 128 + 256))
                mx = jnp.max(s, axis=-1, keepdims=True)
                e = jnp.exp(s - mx)
                p = e * (1.0 / jnp.sum(e, axis=-1, keepdims=True))
                delta = jnp.sum(p * dp, axis=-1, keepdims=True)
                ds = p * (dp - delta)
                ps.append(p.astype(bf16))
                dss.append(ds.astype(bf16))
            return ps, dss

        def kv_grads(b, ps, dss, mid=None):
            t = jnp.concatenate([q[b * sq:(b + 1) * sq], do[b * sq:(b + 1) * sq]], axis=0).T
            for h in range(2):
                if h == 1 and mid is not None:
                    mid()
                th = t[h * dh:(h + 1) * dh]
                lhs = jnp.concatenate([jnp.where(lane_lo_t, th, 0.0),
                                       jnp.where(lane_lo_t, 0.0, th)], axis=0).astype(bf16)
                res = _dot(lhs, jnp.concatenate([dss[h], ps[h]], axis=0))
                dkbuf[slot, b, h * dh:(h + 1) * dh, :] = res[0:dh].astype(bf16)
                dvbuf[slot, b, h * dh:(h + 1) * dh, :] = res[dh:2 * dh].astype(bf16)

        def pv(b, pp, which):
            c0 = _dot_nt(pp[0], kv(which, b, 0, 128))
            c1 = _dot_nt(jnp.concatenate(pp, axis=0), kv(which, b, 128, 256))
            c2 = _dot_nt(pp[1], kv(which, b, 256, 384))
            c1 = jnp.where(lane_lo, c1[0:sq], c1[sq:2 * sq])
            return jnp.concatenate([c0, c1, c2], axis=1)

        o_list = []
        dq_list = []
        nxt = scores(0)
        for b in range(nb):
            ps, dss = nxt
            if b + 1 < nb:
                nxt = scores(b + 1)
                kv_grads(b, ps, dss)
            o_list.append(pv(b, ps, 1))
            dq_list.append(pv(b, dss, 0) * scale)
            point("b%d" % b, o_list[-1][0:16, 0:128],
                  dq_list[-1][0:16, 256:384] if b >= hb else None)
            if b in (hb - 1, nb - 3, nb - 2):
                pl.when(j == jl)(functools.partial(
                    lambda gi: start(last_out(gi)), (hb - 1, nb - 3, nb - 2).index(b)))

        o = jnp.concatenate(o_list, axis=0)
        dq = jnp.concatenate(dq_list, axis=0).astype(bf16)
        t_out = _dot(o.astype(bf16), wo)
        out_acc[rows, :] += t_out
        point("out", t_out[0:16, 384:512], t_out[m - 16:m, 512:640])
        dx_acc[rows, :] += _dot_nt(dq, wq)
        fresh = bg == 0
        dwo_new = jnp.where(fresh, 0.0, dwo_acc[...]) + _dot(o.T.astype(bf16), g)
        dwo_acc[...] = dwo_new
        dwo_st[hp % 2] = dwo_new.astype(bf16)
        point("dwo", dwo_new[0:16, 384:512], dwo_new[d2 - 16:d2, 512:640])
        for lo, hi in ((0, _SPLIT), (_SPLIT, dm)):
            if lo:
                kv_grads(nb - 1, ps, dss,
                         lambda: issue_out(is2 + end_rd, unit(j - 2 + end_rd)))
            dwq_new = jnp.where(fresh, 0.0, dwq_acc[lo:hi, :]) + _dot(xt_sc[bg, lo:hi, :], dq)
            dwq_acc[lo:hi, :] = dwq_new
            dwq_st[hp % 2, lo:hi, :] = dwq_new.astype(bf16)

    def first():
        return [wq_head(0, sem_dw.at[0])] + w_in(0) + kv_in_big(0)

    start(xg_in(0))
    fence()
    start(first())
    fence()
    start(xg_in(1) + kv_in_big(1))
    fence()
    start(wq_bulk())
    fence()

    def zero_rows(i, carry):
        r = pl.ds(pl.multiple_of(i * 64, 64), 64)
        out_acc[r, :] = jnp.zeros((64, dm), f32)
        dx_acc[r, :] = jnp.zeros((64, dm), f32)
        return carry

    jax.lax.fori_loop(0, out_acc.shape[0] // 64, zero_rows, 0)
    dwq_acc[...] = jnp.zeros_like(dwq_acc)
    dwo_acc[...] = jnp.zeros_like(dwo_acc)
    wait(xg_in(0))
    xpose(0)
    wait(first())

    def loop_body(j, carry):
        step_sync(j)
        step_body(j)
        return carry

    jax.lax.fori_loop(0, n_steps, loop_body, 0)

    wait(dw_out(n_hp - 2))
    start(interleave(last_out(3), dw_out(n_hp - 1)))
    fence()
    cast_od(1)
    start(od_out(1))
    wait(kv_out(jl - 3))
    wait(kv_out(jl - 2))
    wait(kv_out(jl - 1))
    wait(last_out(0) + last_out(1) + last_out(2) + last_out(3))
    wait(od_out(0) + od_out(1))
    wait(dw_out(n_hp - 1))


@jax.jit
def pallas_standalone__gqa_block_cached__near_ridge_kernel(
    x: jax.Array,
    k_cache: jax.Array,
    v_cache: jax.Array,
    wq: jax.Array,
    wo: jax.Array,
    grad_out: jax.Array,
):
    B, Sq, D = x.shape
    _, H, Sk, Dh = k_cache.shape
    assert (B, Sq, D, Dh) == (16, 64, 640, 192) and H % 4 == 0 and H >= 8
    assert wq.shape == (D, H * Dh) and wo.shape == (H * Dh, D)
    nb = B // 2
    n_hp = H // 2
    m = nb * Sq
    d2 = 2 * Dh
    bf16 = jnp.bfloat16
    f32 = jnp.float32

    x2 = x.reshape(B * Sq, D)
    g2 = grad_out.reshape(B * Sq, D)
    wo3 = wo.reshape(n_hp, d2, D)
    kt = jnp.swapaxes(k_cache, 2, 3).reshape(B, H * Dh, Sk)
    vt = jnp.swapaxes(v_cache, 2, 3).reshape(B, H * Dh, Sk)

    any_spec = pl.BlockSpec(memory_space=pl.ANY)
    kv_half = pltpu.VMEM((_NSLOT + 1, nb // 2, d2, Sk), bf16)

    out, dx, dkt, dvt, dwq, dwo = pl.pallas_call(
        functools.partial(_kernel, nb=nb, sq=Sq, dh=Dh, scale=float(Dh) ** -0.5, n_hp=n_hp),
        in_specs=[any_spec] * 6,
        out_specs=[any_spec] * 6,
        out_shape=[
            jax.ShapeDtypeStruct((B * Sq, D), bf16),
            jax.ShapeDtypeStruct((B * Sq, D), bf16),
            jax.ShapeDtypeStruct((B, H * Dh, Sk), bf16),
            jax.ShapeDtypeStruct((B, H * Dh, Sk), bf16),
            jax.ShapeDtypeStruct((D, H * Dh), bf16),
            jax.ShapeDtypeStruct((n_hp, d2, D), bf16),
        ],
        scratch_shapes=[
            pltpu.VMEM((B * Sq, D), bf16),
            pltpu.VMEM((B * Sq, D), bf16),
            pltpu.VMEM((2, D, m), bf16),
            pltpu.VMEM((n_hp, D, d2), bf16),
            pltpu.VMEM((2, d2, D), bf16),
            pltpu.VMEM((B * Sq, D), f32),
            pltpu.VMEM((B * Sq, D), f32),
            pltpu.VMEM((D, d2), f32),
            pltpu.VMEM((d2, D), f32),
            pltpu.VMEM((2, D, d2), bf16),
            pltpu.VMEM((2, d2, D), bf16),
            pltpu.VMEM((B * Sq, D), bf16),
            pltpu.VMEM((B * Sq, D), bf16),
            kv_half, kv_half, kv_half, kv_half,
            pltpu.VMEM((_NSLOT, nb, d2, Sk), bf16),
            pltpu.VMEM((_NSLOT, nb, d2, Sk), bf16),
            pltpu.SemaphoreType.DMA((_NSLOT,)),
            pltpu.SemaphoreType.DMA((_NSLOT,)),
            pltpu.SemaphoreType.DMA((1,)),
            pltpu.SemaphoreType.DMA((1,)),
            pltpu.SemaphoreType.DMA((3,)),
            pltpu.SemaphoreType.REGULAR((1,)),
        ],
        compiler_params=pltpu.CompilerParams(
            vmem_limit_bytes=110 * 1024 * 1024,
            disable_bounds_checks=True,
        ),
    )(x2, g2, wq, wo3, kt, vt)

    dk = jnp.swapaxes(dkt.reshape(B, H, Dh, Sk), 2, 3)
    dv = jnp.swapaxes(dvt.reshape(B, H, Dh, Sk), 2, 3)
    return (out.reshape(B, Sq, D), dx.reshape(B, Sq, D), dk, dv, dwq,
            dwo.reshape(H * Dh, D))
```
